```python
import os as _os
_os.environ.setdefault("JAX_PLATFORMS", "cpu")
import jax
import jax.numpy as jnp

def _softmax(x, axis=-1):
    return jax.nn.softmax(x, axis=axis)
def _gelu(x):
    return jax.nn.gelu(x, approximate=True)
def _silu(x):
    return jax.nn.silu(x)
def _sigmoid(x):
    return jax.nn.sigmoid(x)
def _layernorm(x, axis=-1, eps=1e-5):
    m = jnp.mean(x, axis=axis, keepdims=True)
    v = jnp.var(x, axis=axis, keepdims=True)
    return (x - m) / jnp.sqrt(v + eps)
def _scatter_add(tgt, idx, src, axis=0):
    return tgt.at[idx].add(src)
def _segment_sum(src, seg, n):
    return jax.ops.segment_sum(src, seg, n)
class _Rng:
    def __init__(self, key):
        self._k = key
    def _next(self):
        self._k, sub = jax.random.split(self._k)
        return sub
    def normal(self, shape):
        return jax.random.normal(self._next(), shape, dtype=jnp.bfloat16)
    def randint(self, lo, hi, shape):
        return jax.random.randint(self._next(), shape, lo, hi, dtype=jnp.int32)
    def uniform(self, shape, lo=0.0, hi=1.0):
        return jax.random.uniform(self._next(), shape, jnp.bfloat16, lo, hi)
    def permutation(self, n):
        return jax.random.permutation(self._next(), n)


kernel_name = 'gated_mix__ssm_conv_h3__linear_kernel_hedgehog__prompt'

def setup_inputs():
    _rng = _Rng(jax.random.key(int.from_bytes(__import__("os").urandom(4), "little")))
    _w = (lambda a: (lambda t: t.astype(jnp.bfloat16) if jnp.issubdtype(t.dtype, jnp.floating) else t)(jnp.asarray(a)))
    def _A_setup():
        B, S, D = 1, 2048, 576
        ks = 4
        return {
            "q": _w((lambda *s: _rng.normal(s) * 0.05)(B, S, D)),
            "k": _w((lambda *s: _rng.normal(s) * 0.4)(B, S, D)),
            "v": _w((lambda *s: _rng.normal(s) * 0.4)(B, S, D)),
            "shift_k": _w((lambda *s: _rng.normal(s) * 0.4)(D, ks) * 0.5),
            "ssm_k": _w((lambda *s: _rng.normal(s) * 0.4)(D, S) * (1.0 / S ** 0.5)),
            "ssm_D": _w((lambda *s: _rng.normal(s) * 0.4)(D)),
        }
    _A_in = _A_setup()

    def _B_setup():
        B, S, D, H = 1, 2048, 576, 32
        Dh = D // H
        return {
            "x": _w((lambda *s: _rng.normal(s) * 0.05)(B, S, D)),
            "wqkv": _w((lambda *s: _rng.normal(s) * 0.8)(D, 3 * D)),
            "w_phi": _w((lambda *s: _rng.normal(s) * 0.8)(H, Dh, Dh) * (Dh ** -0.5)),
            "wo": _w((lambda *s: _rng.normal(s) * 0.05)(D, D)),
        }
    _B_in = _B_setup()

    return {
        "A_q": _A_in["q"],
        "A_k": _A_in["k"],
        "A_v": _A_in["v"],
        "A_shift_k": _A_in["shift_k"],
        "A_ssm_k": _A_in["ssm_k"],
        "A_ssm_D": _A_in["ssm_D"],
        "B_x": _B_in["x"],
        "B_wqkv": _B_in["wqkv"],
        "B_w_phi": _B_in["w_phi"],
        "B_wo": _B_in["wo"],
        "gate_w": _w((lambda *s: _rng.normal(s) * 0.05)(576) * 16.0),
    }

def reference(A_q, A_k, A_v, A_shift_k, A_ssm_k, A_ssm_D, B_x, B_wqkv, B_w_phi, B_wo, gate_w):
    def _A_ref(q, k, v, shift_k, ssm_k, ssm_D):
        B, S, D = q.shape
        ks = shift_k.shape[-1]
        k_pad = jnp.pad(k, ((0, 0), (ks - 1, 0), (0, 0)))
        k_shift = jnp.zeros_like(k)
        for t in range(ks):
            k_shift = k_shift + k_pad[:, t:t + S, :] * shift_k[:, ks - 1 - t][None, None, :]
        kv = k_shift * v
        L = 2 * S
        kv_pad = jnp.pad(kv, ((0, 0), (0, S), (0, 0)))
        kf_pad = jnp.pad(ssm_k, ((0, 0), (0, S)))
        kv_f = (lambda x, axes=(-2,-1): jnp.fft.rfft2(x.astype(jnp.float32), axes=axes))(kv_pad[:, None, :, :], axes=(1, 2))
        kf_f = (lambda x, axes=(-2,-1): jnp.fft.rfft2(x.astype(jnp.float32), axes=axes))(kf_pad[:, None, :], axes=(1, 2))
        kf_f = (lambda x, *d: x.transpose(*d))(kf_f, 1, 2, 0)
        y_f = kv_f * kf_f[None, :, :, :]
        y = (lambda x, s, axes=(-2,-1): jnp.fft.irfft2(x, s=s, axes=axes).astype(jnp.bfloat16))(y_f, (1, L), axes=(1, 2))[:, 0, :S, :]
        y = y + kv * ssm_D[None, None, :]
        return q * y

    def _B_ref(x, wqkv, w_phi, wo):
        B, S, D = x.shape
        H = 32; Dh = D // H
        qkv = (lambda x, *d: x.transpose(*d))((x @ wqkv).reshape(B, S, 3, H, Dh), 2, 0, 3, 1, 4)
        q, k, v = qkv[0], qkv[1], qkv[2]
        pq = jnp.einsum("bhsd,hdf->bhsf", q, w_phi)
        pk = jnp.einsum("bhsd,hdf->bhsf", k, w_phi)
        phi_q = jnp.concatenate([_softmax(pq, axis=-1), _softmax(-pq, axis=-1)], axis=-1)
        phi_k = jnp.concatenate([_softmax(pk, axis=-1), _softmax(-pk, axis=-1)], axis=-1)
        kv = jnp.einsum("bhsf,bhsd->bhfd", phi_k, v)
        z  = jnp.einsum("bhsf->bhf", phi_k)
        num = jnp.einsum("bhqf,bhfd->bhqd", phi_q, kv)
        den = jnp.einsum("bhqf,bhf->bhq", phi_q, z)[..., None] + 1e-6
        o = num / den
        return (lambda x, *d: x.transpose(*d))(o, 0, 2, 1, 3).reshape(B, S, D) @ wo

    x = A_q
    g = _sigmoid((x * gate_w).sum(-1, keepdims=True))
    a = _A_ref(x, A_k, A_v, A_shift_k, A_ssm_k, A_ssm_D)
    b = _B_ref(x, B_wqkv, B_w_phi, B_wo)
    return g * a + (1 - g) * b
```

```python
import jax
import jax.numpy as jnp
from jax import lax
import jax.experimental.pallas as pl
import jax.experimental.pallas.tpu as pltpu

S, D, H, DH = 2048, 576, 32, 18
NG, GR = 8, 72
PR, PM = 80, 48
NS = 8
CB, NB = 128, 16
NCH = D // 8
KT = 5
NLAST = 4
LOG2E = 1.4426950408889634
f32 = jnp.float32
bf16 = jnp.bfloat16
u32 = jnp.uint32


def _nt(a, b):
    return lax.dot_general(a, b, (((1,), (1,)), ((), ())), preferred_element_type=f32)


def _nn(a, b):
    return jnp.dot(a, b, preferred_element_type=f32)


def _iota(shape, dim):
    return lax.broadcasted_iota(jnp.int32, shape, dim)


def _kw(t):
    return 128 if t < KT - 1 else 64


def _mul(i, m):
    return i * m if isinstance(i, int) else pl.multiple_of(i * m, m)


def _load_lhs(ref, r0, r1):
    return jnp.concatenate(
        [pltpu.bitcast(ref[t, r0 // 2:r1 // 2, 0:_kw(t)], bf16) for t in range(KT)], axis=1)


def _store_lhs(ref, r0, val):
    w = pltpu.bitcast(val, u32)
    for t in range(KT):
        ref[t, r0 // 2:(r0 + val.shape[0]) // 2, 0:_kw(t)] = w[:, 128 * t:128 * t + _kw(t)]


def _row_f_h(rho):
    r, sub = rho >> 3, rho & 7
    f = jnp.where(r == 4, 16 + (sub >> 2), 4 * jnp.where(r > 4, r - 5, r) + (sub >> 1))
    h = jnp.where(r == 4, sub & 3, jnp.where(r > 4, 2, 0) + (sub & 1))
    return f, h


def _recip(t):
    r = pl.reciprocal(t, approx=True)
    return r * (2.0 - t * r)


def _dual_softmax(pg):
    w = pg.shape[-1]
    b1 = (_iota((8, w), 0) & 2) == 0

    def reduce(x, op):
        ma = op(op(x[0], x[1]), op(x[2], x[3]))
        mb = op(op(x[5], x[6]), op(x[7], x[8]))
        e = op(op(jnp.where(b1, ma, mb), x[4]), pltpu.roll(jnp.where(b1, mb, ma), 2, 0))
        return op(e, pltpu.roll(e, 4, 0))

    def spread(f):
        fr = pltpu.roll(f, 2, 0)
        return [jnp.where(b1, f, fr)] * 4 + [f] + [jnp.where(b1, fr, f)] * 4

    p = [pg[8 * r:8 * r + 8] for r in range(9)]
    mx = spread(reduce(p, jnp.maximum))
    mn = spread(reduce(p, jnp.minimum))
    ep = [jnp.exp2(p[r] - mx[r]) for r in range(9)]
    en = [jnp.exp2(mn[r] - p[r]) for r in range(9)]
    rp = spread(_recip(reduce(ep, jnp.add)))
    rn = spread(_recip(reduce(en, jnp.add)))
    ep = [ep[r] * rp[r] for r in range(9)]
    en = [en[r] * rn[r] for r in range(9)]
    return [jnp.concatenate(ep[4 * q:4 * q + 5] + en[4 * q:4 * q + 5], axis=0).astype(bf16) for q in range(2)]


def _slot(blk, which, comp):
    return 8 * (12 * (blk // 2) + 6 * which + 3 * (blk % 2) + comp)


def _kernel(x_hbm, k_hbm, v_hbm, skt_hbm, h_hbm, dsk_hbm, wqkv_hbm, wphi_hbm, wo_hbm, gw_hbm,
            out_hbm,
            uh_s, yf_s, yl_s, phiq_s, in_s, out_s, g_s, wo_s, wot_s, wqkv_s, ft_s, gt_s, wq_s,
            wkv_s, col_s, hc_s, kvt_s, ak_s, skt_s, dsk_s, wphi_s, gw_s, zv_s, zs_s, sem_in,
            sem_w, sem_out, sem_f):
    def start_x(j):
        for c in range(2):
            pltpu.make_async_copy(x_hbm.at[0, :, pl.ds(_mul(2 * j + c, CB), CB)], in_s.at[j, c],
                                  sem_in.at[j]).start()

    def start_hkv(j):
        for c in range(2):
            col = pl.ds(_mul(2 * j - 2 + c, CB), CB)
            for n, src in enumerate((h_hbm.at[:, col], k_hbm.at[0, :, col], v_hbm.at[0, :, col])):
                pltpu.make_async_copy(src, in_s.at[j, 2 + 2 * n + c], sem_in.at[j]).start()

    def wait_set(j, lo=0, hi=8):
        pltpu.make_async_copy(in_s.at[j, lo:hi], in_s.at[j, lo:hi], sem_in.at[j]).wait()

    small = [pltpu.make_async_copy(src, dst, sem_w.at[3 + n]) for n, (src, dst) in
             enumerate(((wphi_hbm, wphi_s), (skt_hbm, skt_s), (dsk_hbm, dsk_s), (gw_hbm, gw_s)))]
    wq_cp = pltpu.make_async_copy(wqkv_hbm.at[:, 0:640], wqkv_s.at[:, 0:640], sem_w.at[0])
    wkv_cp = pltpu.make_async_copy(wqkv_hbm.at[:, 640:3 * D], wqkv_s.at[:, 640:3 * D], sem_w.at[1])
    wo_cp = pltpu.make_async_copy(wo_hbm, wo_s.at[0:D, :], sem_w.at[2])

    def fence():
        pl.semaphore_signal(sem_f, 1)
        pl.semaphore_wait(sem_f, 1)

    for cp in small:
        cp.start()
    fence()
    wq_cp.start()
    fence()
    start_x(0)

    zs_s[0] = 0
    zv_s[...] = jnp.zeros(zv_s.shape, jnp.int32)

    idx = (_iota((CB, CB), 0) * (4 * _iota((CB, CB), 1) + 1)) & 511
    ang = idx.astype(f32) * (3.141592653589793 / 256.0)
    fc = jnp.cos(ang).astype(bf16)
    fs = (-jnp.sin(ang)).astype(bf16)
    ft_s[0] = pltpu.bitcast(fc, u32)
    ft_s[1] = pltpu.bitcast(fs, u32)
    gt_s[0] = pltpu.bitcast(fc.T, u32)
    gt_s[1] = pltpu.bitcast(fs.T, u32)

    in_s[0, 5] = jnp.zeros((D, CB), bf16)
    hc_s[0] = jnp.zeros((D, CB), f32)
    kvt_s[...] = jnp.zeros(kvt_s.shape, f32)
    wo_s[D:640, :] = jnp.zeros((640 - D, D), bf16)

    for cp in small:
        cp.wait()
    start_hkv(1)
    start_x(1)

    e18 = _iota((H, 640), 1) - DH * _iota((H, 640), 0)
    bmat = None
    for d in range(DH):
        t = _nn(wphi_s[d], jnp.where(e18 == d, 1.0, 0.0).astype(bf16))
        bmat = t if bmat is None else bmat + t
    expand = jnp.where(_row_f_h(_iota((80, DH), 0))[0] == _iota((80, DH), 1), 1.0, 0.0).astype(bf16)
    a_q = _nn(expand, bmat.astype(bf16))

    def make_fold(a_all, off, lane0, dst):
        acc = {}
        span = lambda v: (off + GR * (v // 9) + (36 if v % 9 > 4 else 0),
                          off + GR * (v // 9) + (36 if v % 9 < 4 else GR))
        last = {v: (span(v)[1] - 1) // 128 for v in range(NCH)}
        st = dict(done=0)

        def run(tiles):
            for t in tiles:
                vs = [v for v in range(NCH) if span(v)[0] < 128 * (t + 1) and span(v)[1] > 128 * t]
                v0, v1 = vs[0], vs[-1] + 1
                pad = (v1 - v0) % 2
                parts = []
                for g in range(v0 // 9, (v1 - 1) // 9 + 1):
                    a, b = max(v0, 9 * g) - 9 * g, min(v1, 9 * g + 9) - 9 * g
                    b += pad if g == (v1 - 1) // 9 else 0
                    shp = (8 * (b - a), 128)
                    col = _iota(shp, 1) + 128 * t
                    c0 = off + GR * g + DH * _row_f_h(_iota(shp, 0) + 8 * a)[1]
                    parts.append(jnp.where((col >= c0) & (col < c0 + DH),
                                           a_all[8 * a:8 * b, 128 * t:128 * (t + 1)], 0.0))
                lhs = jnp.concatenate(parts, axis=0).astype(bf16)
                r = _nt(lhs, wqkv_s[:, lane0 + 128 * t:lane0 + 128 * (t + 1)])
                for v in range(v0, v1):
                    p = r[8 * (v - v0):8 * (v - v0) + 8]
                    acc[v] = p if v not in acc else acc[v] + p
                ready = st["done"]
                while ready < NCH and last[ready] <= t:
                    ready += 1
                ready -= (ready - st["done"]) % 2
                if ready > st["done"]:
                    w = jnp.concatenate([acc.pop(v) for v in range(st["done"], ready)], axis=0) * LOG2E
                    _store_lhs(dst, 8 * st["done"], w.astype(bf16))
                    st["done"] = ready

        return run

    def wide(ref, axis):
        return jnp.concatenate([pltpu.bitcast(ref[0], bf16), pltpu.bitcast(ref[1], bf16)], axis=axis)

    def conv_work(dst, chunks, pairs, back, delay=False):
        never = zv_s[...] != 0
        zi = zs_s[0]
        tok = None
        first = True
        if delay:
            tok = [pltpu.roll(pltpu.bitcast(zv_s[...], f32), 1, 1)] * 2
        for ch in chunks:
            k1 = {}
            for comp in range(3):
                uw, hw = {}, {}
                for n, p in enumerate(pairs):
                    a0 = 2 * p
                    acc = list(k1[p]) if comp else [None, None]
                    hist = [[], []]
                    for b in range(a0 + 2):
                        if b not in uw:
                            uw[b] = uh_s[ch, _slot(b, 0, comp):_slot(b, 0, comp) + 8, :]
                        for t in range(2):
                            m = a0 + t - b
                            if m < 0:
                                continue
                            if m not in hw:
                                hw[m] = uh_s[ch, _slot(m, 1, comp):_slot(m, 1, comp) + 8, :]
                            k = uw[b] * hw[m]
                            if b == 0 and tok is not None:
                                k = jnp.where(never, tok[t], k)
                            if b == 1 and t == 1 and n == 0 and not first and comp != 1:
                                mt = dst[chunks[0] + zi, 64 * pairs[0] + 16:64 * pairs[0] + 32, :]
                                k = jnp.where(never, mt.astype(f32)[0:8], k)
                            if acc[t] is None:
                                acc[t] = k
                            else:
                                acc[t] = acc[t] - k if comp == 2 else acc[t] + k
                            hist[t].append(acc[t])
                    tok = [h[max(len(h) - 1 - back, 0)] for h in hist]
                    first = False
                    if comp == 0:
                        k1[p] = acc
                    else:
                        r0 = 64 * p + (16 if comp == 1 else 0)
                        dst[ch, r0:r0 + 16, :] = jnp.concatenate(acc, axis=0).astype(bf16)

    def qpart(i, c, nsl=1):
        cuts = [n * (D // nsl) for n in range(nsl)] + [D + 16]
        pq = jnp.concatenate([_nn(_load_lhs(wq_s, a, b), in_s[i, c]) for a, b in zip(cuts[:-1], cuts[1:])], axis=0)
        for g in range(NG):
            ph = _dual_softmax(pq[GR * g:GR * (g + 1)])
            for q in range(2):
                phiq_s[2 * i + c, PR * (2 * g + q):PR * (2 * g + q + 1), :] = ph[q]
        g_s[i, 8 * c:8 * c + 8, :] = jax.nn.sigmoid(pq[D:D + 8])

    def dft_step(i, order, other):
        base = _mul(i, 96)

        def put(c, which, comp, val):
            uh_s[:, pl.ds(base + _slot(c, which, comp), 8), :] = val.reshape(NCH, 8, CB)

        st = dict(pc=None, pd=None)

        def hpart(c):
            pc, pd = (hc_s[0], hc_s[1]) if c == 0 else (st["pc"], st["pd"])
            hf = _nn(in_s[i + 1, 2 + c], wide(ft_s, 1))
            cc, dd = hf[:, 0:CB], hf[:, CB:2 * CB]
            c1 = cc - pd
            d1 = dd + pc
            put(c, 1, 0, c1)
            put(c, 1, 1, d1 - c1)
            put(c, 1, 2, c1 + d1)
            st["pc"], st["pd"] = cc, dd
            if c == 1 and not (isinstance(i, int) and i == NS - 1):
                hc_s[0] = cc
                hc_s[1] = dd

        lane = _iota((D // 2, CB), 1)
        kp = [pltpu.bitcast(in_s[i, 5], u32)]
        kp += [pltpu.bitcast(in_s[i + 1, 4 + c], u32) for c in range(2)]
        ut = []
        for c in range(2):
            ks = in_s[i + 1, 4 + c].astype(f32) * col_s[0]
            for j in range(1, 4):
                kj = pltpu.roll(jnp.where(lane >= CB - j, kp[c], kp[c + 1]), j, 1)
                ks = ks + pltpu.bitcast(kj, bf16).astype(f32) * col_s[j]
            ut.append(ks * in_s[i + 1, 6 + c].astype(f32))

        def upart(c):
            uf = _nn(ut[c].astype(bf16), wide(ft_s, 1))
            aa, bb = uf[:, 0:CB], uf[:, CB:2 * CB]
            put(c, 0, 0, aa + bb)
            put(c, 0, 1, aa)
            put(c, 0, 2, bb)

        for tkn in order.split():
            {"h": hpart, "u": upart}.get(tkn[0], other)(int(tkn[1]))

    wq_cp.wait()
    start_hkv(2)
    start_x(2)
    make_fold(a_q, 0, 0, wq_s)(range(KT))
    ak_s[...] = pltpu.roll(a_q, 64, 1)
    for j in range(4):
        col_s[j] = jnp.broadcast_to(skt_s[j:j + 1, :], (CB, D)).T.astype(f32)
    hc_s[1] = -jnp.broadcast_to(dsk_s[...].reshape(1, D), (CB, D)).T.astype(f32)
    _store_lhs(wq_s, D, jnp.broadcast_to(gw_s[...].reshape(1, D), (16, D)))
    wait_set(0, 0, 2)
    qpart(0, 0, 2)
    qpart(0, 1, 2)
    start_hkv(3)
    start_x(3)

    def phase1(i, carry):
        wait_set(i + 1)
        dft_step(i, "q0 u0 q1 u1 h0 h1", lambda c: qpart(i + 1, c))

        @pl.when(i + 4 <= NS)
        def _():
            start_hkv(i + 4)

        @pl.when(i + 4 < NS)
        def _():
            start_x(i + 4)

        @pl.when(i == NS - 4)
        def _():
            wkv_cp.start()

        @pl.when(i == NS - 3)
        def _():
            wo_cp.start()

        return carry

    lax.fori_loop(0, NS - 1, phase1, 0)

    wait_set(NS, 2, 8)
    wkv_cp.wait()
    _store_lhs(wkv_s, D, wqkv_s[:, 2 * D:3 * D].T)
    make_fold(ak_s, 64, 512, wkv_s)(range(KT))
    dft_step(NS - 1, "h0 h1 u0 u1", None)
    wo_cp.wait()

    def phase2(i, carry):
        conv_work(yf_s, [i * 18 + j for j in range(18)], list(range(6)), 2, True)
        for n in range(2):
            t = jnp.minimum(2 * i + n, KT - 1)
            wot_s[t] = pltpu.bitcast(wo_s[pl.ds(pl.multiple_of(t * 128, 128), 128), :].T, u32)

        vt = [_nn(_load_lhs(wkv_s, D, 2 * D), in_s[2 * i + c // 2, c % 2]) for c in range(4)]
        pk = [_nn(_load_lhs(wkv_s, 0, D), in_s[2 * i + c // 2, c % 2]) for c in range(4)]
        ones = jnp.ones((8, 2 * CB), f32)
        for n in range(2):
            pk2 = jnp.concatenate(pk[2 * n:2 * n + 2], axis=1)
            vt2 = jnp.concatenate(vt[2 * n:2 * n + 2], axis=1)
            for g in range(NG):
                ph = _dual_softmax(pk2[GR * g:GR * (g + 1)])
                for q in range(2):
                    r0 = GR * g + 32 * q
                    vg = jnp.concatenate([vt2[r0:r0 + 40], ones], axis=0).astype(bf16)
                    kvt_s[2 * g + q] = kvt_s[2 * g + q] + _nt(vg, ph[q])
        return carry

    lax.fori_loop(0, 4, phase2, 0)

    def masked_state():
        rr = _iota((PM, PR), 0)
        cc = _iota((PM, PR), 1)
        out = {}
        for q in range(2):
            ch = _row_f_h(32 * q + jnp.where(cc >= 40, cc - 40, cc))[1]
            vr = rr + 32 * q
            keep = ((((vr >= DH * ch) & (vr < DH * ch + DH)) & (rr < 40))
                    | ((rr >= 40 + 2 * ch) & (rr < 42 + 2 * ch)))
            keep = keep & ((ch >> 1) == q)
            for g in range(NG):
                out[2 * g + q] = jnp.where(keep, kvt_s[2 * g + q], 0.0).astype(bf16)
        return out

    def out_copy(t, r0=0, r1=D, n=0):
        return pltpu.make_async_copy(out_s.at[t, r0:r1], out_hbm.at[0, r0:r1, pl.ds(_mul(t, CB), CB)],
                                     sem_out.at[t + n])

    def phase3(b0, ysrc, chunks, order):
        sub = _iota((8, CB), 0)
        res = {}
        conv_work(yl_s, chunks, [6, 7], 0)
        kvb = masked_state()

        def num(c):
            i, cc = b0 + c // 2, c % 2
            gate = g_s[i, 8 * cc:8 * cc + 8, :]
            os_ = []
            for g in range(NG):
                ra, rb = [_nn(kvb[2 * g + q], phiq_s[2 * i + cc, PR * (2 * g + q):PR * (2 * g + q + 1), :])
                          for q in range(2)]
                r = jnp.concatenate([ra[0:32], ra[32:40] + rb[0:8], rb[8:40]], axis=0)
                sc = (1.0 - gate) / (ra[40:48] + rb[40:48] + 1e-6)
                b = [jnp.broadcast_to(sc[2 * h:2 * h + 1], (8, CB)) for h in range(4)]
                pat = [b[0], b[0], jnp.where(sub < 2, b[0], b[1]), b[1], jnp.where(sub < 4, b[1], b[2]),
                       b[2], jnp.where(sub < 6, b[2], b[3]), b[3], b[3]]
                os_.append(r * jnp.concatenate(pat, axis=0))
            res["o%d" % c] = jnp.concatenate(os_, axis=0).astype(bf16)

        def inv(n):
            yb = _mul(b0 + n, 64)
            yf = jnp.concatenate([ysrc[:, pl.ds(yb + 16 * c, 16), :].reshape(2 * D, CB) for c in range(2)], axis=1)
            res["y%d" % n] = _nn(yf, wide(gt_s, 0)).reshape(NCH, 2, 8, CB)

        def wo(c):
            i, cc = b0 + c // 2, c % 2
            gate = g_s[i, 8 * cc:8 * cc + 8, :] * (1.0 / 128.0)
            xt = in_s[i, cc].astype(f32)
            ay = (xt.reshape(NCH, 8, CB) * gate[None] * res["y%d" % (c // 2)][:, cc]).reshape(D, CB)
            bt = _nn(_load_lhs(wot_s, 0, D), res["o%d" % c])
            res_t = (ay + bt).astype(bf16)
            if isinstance(i, int) and 2 * i + cc == NB - 1:
                for n in range(NLAST):
                    r0, r1 = n * (D // NLAST), (n + 1) * (D // NLAST)
                    out_s[NB - 1, r0:r1] = res_t[r0:r1]
                    out_copy(NB - 1, r0, r1, n).start()
            else:
                out_s[2 * i + cc] = res_t
                out_copy(2 * i + cc).start()

        for tkn in order.split():
            {"n": num, "y": inv, "w": wo}[tkn[0]](int(tkn[1]))

    def phase3a(ii, carry):
        phase3(3 * ii, yf_s, [ii * 36 + j for j in range(36)], "y0 n0 n1 y1 n2 n3 y2 n4 n5 w0 w1 w2 w3 w4 w5")
        return carry

    lax.fori_loop(0, 2, phase3a, 0)
    phase3(6, yl_s, [], "y0 n0 n1 n2 n3 w0 w1 y1 w2 w3")
    for t in range(NB - 1):
        out_copy(t).wait()
    for n in range(NLAST):
        out_copy(NB - 1, n * (D // NLAST), (n + 1) * (D // NLAST), n).wait()


@jax.jit
def pallas_gated_mix__ssm_conv_h3__linear_kernel_hedgehog__prompt_kernel(A_q, A_k, A_v, A_shift_k, A_ssm_k, A_ssm_D, B_x, B_wqkv, B_w_phi, B_wo, gate_w):
    del B_x
    hbm = pl.BlockSpec(memory_space=pltpu.HBM)
    scratch = [
        pltpu.VMEM((NCH, 96 * 8, CB), f32),
        pltpu.VMEM((NCH, 64 * NS, CB), bf16),
        pltpu.VMEM((NCH, 64 * NS, CB), bf16),
        pltpu.VMEM((NB, 16 * PR, CB), bf16),
        pltpu.VMEM((NS + 1, 8, D, CB), bf16),
        pltpu.VMEM((NB, D, CB), bf16),
        pltpu.VMEM((NS, 32, CB), f32),
        pltpu.VMEM((640, D), bf16),
        pltpu.VMEM((KT, D // 2, 128), u32),
        pltpu.VMEM((D, 3 * D), bf16),
        pltpu.VMEM((2, CB // 2, CB), u32),
        pltpu.VMEM((2, CB // 2, CB), u32),
        pltpu.VMEM((KT, 320, 128), u32),
        pltpu.VMEM((KT, D, 128), u32),
        pltpu.VMEM((4, D, CB), f32),
        pltpu.VMEM((2, D, CB), f32),
        pltpu.VMEM((2 * NG, PM, PR), f32),
        pltpu.VMEM((80, 640), f32),
        pltpu.VMEM((4, D), bf16),
        pltpu.VMEM((D,), bf16),
        pltpu.VMEM((DH, DH, H), bf16),
        pltpu.VMEM((D,), bf16),
        pltpu.VMEM((8, CB), jnp.int32),
        pltpu.SMEM((1,), jnp.int32),
        pltpu.SemaphoreType.DMA((NS + 1,)),
        pltpu.SemaphoreType.DMA((7,)),
        pltpu.SemaphoreType.DMA((NB + NLAST,)),
        pltpu.SemaphoreType.REGULAR,
    ]
    tr = lambda a: jnp.transpose(a, (0, 2, 1))
    out_t = pl.pallas_call(
        _kernel,
        out_shape=jax.ShapeDtypeStruct((1, D, S), bf16),
        in_specs=[hbm] * 10,
        out_specs=hbm,
        scratch_shapes=scratch,
        compiler_params=pltpu.CompilerParams(vmem_limit_bytes=100 * 2**20,
                                             disable_bounds_checks=True, disable_semaphore_checks=True,
                                             internal_scratch_in_bytes=65536),
        name="gated_mix",
    )(tr(A_q), tr(A_k), tr(A_v), A_shift_k.T, A_ssm_k, A_ssm_D, B_wqkv,
      jnp.transpose(B_w_phi, (1, 2, 0)), B_wo, gate_w)
    return tr(out_t)
```
